```python
import jax
import jax.numpy as jnp

def _softmax(x, axis=-1):
    return jax.nn.softmax(x, axis=axis)
def _gelu(x):
    return jax.nn.gelu(x, approximate=True)
def _silu(x):
    return jax.nn.silu(x)
def _sigmoid(x):
    return jax.nn.sigmoid(x)
def _layernorm(x, axis=-1, eps=1e-5):
    m = jnp.mean(x, axis=axis, keepdims=True)
    v = jnp.var(x, axis=axis, keepdims=True)
    return (x - m) / jnp.sqrt(v + eps)
def _scatter_add(tgt, idx, src, axis=0):
    return tgt.at[idx].add(src)
def _segment_sum(src, seg, n):
    return jax.ops.segment_sum(src, seg, n)
class _Rng:
    def __init__(self, key):
        self._k = key
    def _next(self):
        self._k, sub = jax.random.split(self._k)
        return sub
    def normal(self, shape):
        return jax.random.normal(self._next(), shape, dtype=jnp.bfloat16)
    def randint(self, lo, hi, shape):
        return jax.random.randint(self._next(), shape, lo, hi, dtype=jnp.int32)
    def uniform(self, shape, lo=0.0, hi=1.0):
        return jax.random.uniform(self._next(), shape, jnp.bfloat16, lo, hi)
    def permutation(self, n):
        return jax.random.permutation(self._next(), n)


kernel_name = 'standalone__groupnorm__prompt'

def setup_inputs():
    _rng = _Rng(jax.random.key(int.from_bytes(__import__("os").urandom(4), "little")))
    _w = (lambda a: (lambda t: t.astype(jnp.bfloat16) if jnp.issubdtype(t.dtype, jnp.floating) else t)(jnp.asarray(a)))
    B = 2
    G = 32
    cpg = max(1, 1024 // G)
    C = G * cpg
    H, W = 32, 2048
    return {
        "x": _w((lambda *s: _rng.normal(s) * 0.05)(B, C, H, W)),
        "g": _w((lambda *s: _rng.normal(s) * 0.05)(C) + 1.0),
        "b": _w((lambda *s: _rng.normal(s) * 0.05)(C)),
    }

def reference(x, g, b):
    G = 32
    B, C, H, W = x.shape[0], x.shape[1], x.shape[2], x.shape[3]
    xr = x.reshape(B, G, C // G, H, W)
    mu = xr.mean(axis=(2, 3, 4), keepdims=True)
    var = ((xr - mu) ** 2).mean(axis=(2, 3, 4), keepdims=True)
    xn = (xr - mu) / jnp.sqrt(var + 1e-5)
    xn = xn.reshape(B, C, H, W)
    return xn * g[None, :, None, None] + b[None, :, None, None]
```

```python
import functools
import numpy as np
import jax, jax.numpy as jnp
from jax import lax
import jax.experimental.pallas as pl
import jax.experimental.pallas.tpu as pltpu

G = 32
EPS = 1e-5

def make(NP=8, rrows=8, rl=512, wrows=8, wl=2048, gmode='8x128', tail_r=0, tail_w=0):
    def f(x, g, b):
        B, C, H, W = x.shape
        cpg = C // G
        S = 4; cps = cpg // S
        npair = B * G // 2
        nph = npair // NP
        inv_n = 1.0 / (cpg * H * W)
        xv = x.reshape(npair, 2, S, cps, H, W)
        NSTEP = 32

        def kern(x_hbm, g_hbm, b_hbm, o_hbm, buf, gb_v, gb_f, gb_s, rsem, wsem, gsem):
            def issue(rd, pair, slot, step, sem):
                rows, lw = (rrows, rl) if rd else (wrows, wl)
                ch = step // 4
                sub = step - ch * 4
                if rows == 8:
                    r0 = pl.multiple_of(sub * 8, 8); l0 = 0; span = W
                else:
                    r0 = pl.multiple_of((sub // 2) * 16, 16); l0 = pl.multiple_of((sub % 2) * (W // 2), W // 2); span = W // 2
                for l in range(span // lw):
                    for q in range(2):
                        ix = (q, slice(None), ch, pl.ds(r0, rows), pl.ds(l0 + l * lw, lw))
                        if rd:
                            pltpu.make_async_copy(x_hbm.at[(pair,) + ix], buf.at[(slot,) + ix], sem).start(priority=q)
                        else:
                            pltpu.make_async_copy(buf.at[(slot,) + ix], o_hbm.at[(pair,) + ix], sem).start(priority=q)

            def issue_all(rd, pair, slot, sem):
                def body(s, _):
                    issue(rd, pair, slot, s, sem)
                    return 0
                lax.fori_loop(0, NSTEP, body, 0)

            def process(pair, slot, dma):
                def group(q, _):
                    zero = jnp.zeros((8, 128), jnp.float32)
                    def tiles(s, c):
                        for t in range(W // 128):
                            v = buf[slot, q, s, c, :, t * 128:(t + 1) * 128].astype(jnp.float32)
                            yield t, v
                    def sum_body(s, acc):
                        dma(q * 16 + s)
                        def inner(c, acc):
                            acc = list(acc)
                            for _, v in tiles(s, c):
                                for u in range(H // 8):
                                    acc[u] = acc[u] + v[u * 8:(u + 1) * 8]
                            return tuple(acc)
                        return lax.fori_loop(0, cps, inner, acc)
                    acc = lax.fori_loop(0, S, sum_body, (zero,) * (H // 8))
                    tot = functools.reduce(jnp.add, acc)
                    mu = jnp.broadcast_to(jnp.sum(tot, keepdims=True) * inv_n, (8, 128))
                    def var_body(s, acc):
                        dma(q * 16 + 4 + s)
                        def inner(c, acc):
                            acc = list(acc)
                            for _, v in tiles(s, c):
                                for u in range(H // 8):
                                    d = v[u * 8:(u + 1) * 8] - mu
                                    acc[u] = acc[u] + d * d
                            return tuple(acc)
                        return lax.fori_loop(0, cps, inner, acc)
                    acc = lax.fori_loop(0, S, var_body, (zero,) * (H // 8))
                    tot = functools.reduce(jnp.add, acc)
                    var = jnp.sum(tot, keepdims=True) * inv_n
                    rstd = jnp.broadcast_to(lax.rsqrt(var + EPS), (1, 128))
                    mu1 = mu[:1]
                    c0 = ((pair * 2 + q) % G) * cpg
                    def norm_body(h, _):
                        dma(q * 16 + 8 + h)
                        s = h // 2
                        def inner(cc, _):
                            c = (h % 2) * (cps // 2) + cc
                            cg = c0 + s * cps + c
                            a = rstd * gb_s[0, cg // 128, cg % 128]
                            bb = gb_s[1, cg // 128, cg % 128]
                            for t, v in tiles(s, c):
                                buf[slot, q, s, c, :, t * 128:(t + 1) * 128] = ((v - mu1) * a + bb).astype(buf.dtype)
                            return 0
                        return lax.fori_loop(0, cps // 2, inner, 0)
                    lax.fori_loop(0, 2 * S, norm_body, 0)
                    return 0
                lax.fori_loop(0, 2, group, 0)

            def wait_slot(slot, sem):
                pltpu.make_async_copy(buf.at[slot], buf.at[slot], sem).wait()

            def phase(ph, _):
                base = ph * NP
                def rd(j, _):
                    issue_all(True, base + j, j, rsem.at[j])
                    @pl.when((ph == 0) & (j == 0))
                    def _():
                        cg = pltpu.make_async_copy(g_hbm, gb_v.at[0], gsem.at[0])
                        cb = pltpu.make_async_copy(b_hbm, gb_v.at[1], gsem.at[1])
                        cg.start(); cb.start()
                    @pl.when((ph == 0) & (j == 1))
                    def _():
                        pltpu.make_async_copy(g_hbm, gb_v.at[0], gsem.at[0]).wait()
                        pltpu.make_async_copy(b_hbm, gb_v.at[1], gsem.at[1]).wait()
                        gb_f[...] = gb_v[...].astype(jnp.float32)
                        pltpu.make_async_copy(gb_f, gb_s, gsem.at[0]).start()
                    @pl.when((ph == 0) & (j == 2))
                    def _():
                        pltpu.make_async_copy(gb_f, gb_s, gsem.at[0]).wait()
                    return 0
                lax.fori_loop(0, NP - 1, rd, 0)
                def mid(j, _):
                    @pl.when(j == 1)
                    def _():
                        for k in range(1, NP):
                            wait_slot(k, rsem.at[k])
                    @pl.when(j == 0)
                    def _():
                        wait_slot(0, rsem.at[0])
                    def dma(step):
                        @pl.when(j == 0)
                        def _():
                            issue(True, base + NP - 1, NP - 1, step, rsem.at[NP - 1])
                        @pl.when(j > 0)
                        def _():
                            issue(False, base + j - 1, j - 1, step, wsem.at[0])
                    process(base + j, j, dma)
                    return 0
                lax.fori_loop(0, NP, mid, 0)
                issue_all(False, base + NP - 1, NP - 1, wsem.at[0])
                pltpu.make_async_copy(buf, buf, wsem.at[0]).wait()
                return 0
            lax.fori_loop(0, nph, phase, 0)

        gs = (C // 128, 128)
        o = pl.pallas_call(
            kern,
            in_specs=[pl.BlockSpec(memory_space=pltpu.HBM)] * 3,
            out_specs=pl.BlockSpec(memory_space=pltpu.HBM),
            out_shape=jax.ShapeDtypeStruct(xv.shape, x.dtype),
            scratch_shapes=[pltpu.VMEM((NP,) + xv.shape[1:], x.dtype),
                            pltpu.VMEM((2,) + gs, g.dtype), pltpu.VMEM((2,) + gs, jnp.float32), pltpu.SMEM((2,) + gs, jnp.float32),
                            pltpu.SemaphoreType.DMA((NP,)), pltpu.SemaphoreType.DMA((1,)), pltpu.SemaphoreType.DMA((2,))],
            compiler_params=pltpu.CompilerParams(vmem_limit_bytes=124 << 20, disable_bounds_checks=True),
        )(xv, g.reshape(gs), b.reshape(gs))
        return o.reshape(x.shape)
    return f


_impl = make(8)


@jax.jit
def pallas_standalone__groupnorm__prompt_kernel(x: jax.Array, g: jax.Array, b: jax.Array):
    return _impl(x, g, b)
```

```python
import functools
import numpy as np
import jax, jax.numpy as jnp
from jax import lax
import jax.experimental.pallas as pl
import jax.experimental.pallas.tpu as pltpu

G = 32
EPS = 1e-5

def make(phases=(8, 8, 8, 8), rl=512, wl=2048, wq=(0, 1), unroll=2, do_dma=True, do_comp=True, tail_r=0, tail_w=0, nobc=True):
    def f(x, g, b):
        B, C, H, W = x.shape
        cpg = C // G
        S = 4; cps = cpg // S
        npair = B * G // 2
        assert sum(phases) == npair
        NP = max(phases)
        inv_n = 1.0 / (cpg * H * W)
        xv = x.reshape(npair, 2, S, cps, H, W)
        NSTEP = 32

        def kern(x_hbm, g_hbm, b_hbm, o_hbm, buf, gb_v, gb_f, gb_s, rsem, wsem, gsem):
            def issue(rd, pair, slot, lo, hi, sem):
                if not do_dma: return
                def body(step, _):
                    lw = rl if rd else wl
                    ch = step // 4
                    r0 = pl.multiple_of((step - ch * 4) * 8, 8)
                    for l in range(W // lw):
                        for q in range(2):
                            ix = (q, slice(None), ch, pl.ds(r0, 8), pl.ds(l * lw, lw))
                            if rd:
                                pltpu.make_async_copy(x_hbm.at[(pair,) + ix], buf.at[(slot,) + ix], sem).start(priority=q)
                            else:
                                pltpu.make_async_copy(buf.at[(slot,) + ix], o_hbm.at[(pair,) + ix], sem).start(priority=wq[q])
                    return 0
                lax.fori_loop(lo, hi, body, 0)

            def wait_steps(slot, lo, hi, sem):
                if not do_dma: return
                n = hi - lo
                if n // 4:
                    r = buf.at[slot, :, :, pl.ds(0, n // 4)]
                    pltpu.make_async_copy(r, r, sem).wait()
                if n % 4:
                    r = buf.at[slot, :, :, 0, pl.ds(0, (n % 4) * 8)]
                    pltpu.make_async_copy(r, r, sem).wait()

            def process(pair, slot, hook):
                def group(q, _):
                    zero = jnp.zeros((8, 128), jnp.float32)
                    def tiles(c):
                        s = c // cps; cc = c - s * cps
                        for t in range(W // 128):
                            ix = (slot, q, s, cc, slice(None), slice(t * 128, (t + 1) * 128))
                            yield ix, buf[ix].astype(jnp.float32)
                    hook(q * 3)
                    if not do_comp:
                        hook(q * 3 + 1); hook(q * 3 + 2)
                        return 0
                    def sum_body(c, acc):
                        acc = list(acc)
                        for _, v in tiles(c):
                            for u in range(H // 8):
                                acc[u] = acc[u] + v[u * 8:(u + 1) * 8]
                        return tuple(acc)
                    acc = lax.fori_loop(0, cpg, sum_body, (zero,) * (H // 8), unroll=unroll)
                    tot = functools.reduce(jnp.add, acc)
                    mu = jnp.broadcast_to(jnp.sum(tot, keepdims=True) * inv_n, (8, 128))
                    hook(q * 3 + 1)
                    def var_body(c, acc):
                        acc = list(acc)
                        for _, v in tiles(c):
                            for u in range(H // 8):
                                d = v[u * 8:(u + 1) * 8] - mu
                                acc[u] = acc[u] + d * d
                        return tuple(acc)
                    acc = lax.fori_loop(0, cpg, var_body, (zero,) * (H // 8), unroll=unroll)
                    tot = functools.reduce(jnp.add, acc)
                    var = jnp.sum(tot, keepdims=True) * inv_n
                    rstd = jnp.broadcast_to(lax.rsqrt(var + EPS), (1, 128))
                    mu1 = mu[:1]
                    c0 = ((pair * 2 + q) % G) * cpg
                    hook(q * 3 + 2)
                    def norm_body(c, _):
                        cg = c0 + c
                        a = rstd * gb_s[0, cg // 128, cg % 128]
                        bb = gb_s[1, cg // 128, cg % 128]
                        for ix, v in tiles(c):
                            buf[ix] = ((v - mu1) * a + bb).astype(buf.dtype)
                        return 0
                    lax.fori_loop(0, cpg, norm_body, 0, unroll=unroll)
                    return 0
                lax.fori_loop(0, 2, group, 0)

            cg = pltpu.make_async_copy(g_hbm, gb_v.at[0], gsem.at[0])
            cb = pltpu.make_async_copy(b_hbm, gb_v.at[1], gsem.at[1])
            cs = pltpu.make_async_copy(gb_f, gb_s, gsem.at[0])

            def phase(ph, base):
                n = jnp.int32(phases[0])
                for k in range(1, len(phases)):
                    if phases[k] != phases[k - 1]:
                        n = jnp.where(ph >= k, phases[k], n)
                def rd(j, _):
                    issue(True, base + j, j, 0, NSTEP, rsem.at[jnp.minimum(j, 1)])
                    @pl.when(ph == 0)
                    def _():
                        @pl.when(j == 0)
                        def _():
                            cg.start(); cb.start()
                        @pl.when(j == 1)
                        def _():
                            cg.wait(); cb.wait()
                            gb_f[...] = gb_v[...].astype(jnp.float32)
                            cs.start()
                        @pl.when(j == 2)
                        def _():
                            cs.wait()
                    if tail_w:
                        @pl.when((ph > 0) & (j == 0))
                        def _():
                            wait_steps(0, 0, tail_w, wsem.at[1])
                    return 0
                lax.fori_loop(0, n - 1, rd, 0)
                wait_steps(0, 0, NSTEP, rsem.at[0])
                nr = NSTEP - tail_r
                def mid(j, _):
                    def hook(k):
                        @pl.when(j == 0)
                        def _():
                            issue(True, base + n - 1, n - 1, (k * nr) // 6, ((k + 1) * nr) // 6, rsem.at[1])
                    process(base + j, j, hook)
                    @pl.when(j == 0)
                    def _():
                        if tail_r:
                            issue(True, base + n - 1, n - 1, nr, NSTEP, rsem.at[0])
                        def w(k, _):
                            wait_steps(0, 0, NSTEP, rsem.at[1])
                            return 0
                        lax.fori_loop(0, n - 2, w, 0)
                        wait_steps(0, 0, nr, rsem.at[1])
                    nw = jnp.where(j == n - 1, NSTEP - tail_w, NSTEP) if tail_w else NSTEP
                    issue(False, base + j, j, 0, nw, wsem.at[0])
                    if tail_r:
                        @pl.when(j == 0)
                        def _():
                            wait_steps(0, 0, tail_r, rsem.at[0])
                    return 0
                lax.fori_loop(0, n, mid, 0)
                if tail_w:
                    issue(False, base + n - 1, n - 1, NSTEP - tail_w, NSTEP, wsem.at[1])
                def w(k, _):
                    wait_steps(0, 0, NSTEP, wsem.at[0])
                    return 0
                lax.fori_loop(0, n - 1, w, 0)
                wait_steps(0, 0, NSTEP - tail_w, wsem.at[0])
                return base + n
            lax.fori_loop(0, len(phases), phase, jnp.int32(0))
            if tail_w:
                wait_steps(0, 0, tail_w, wsem.at[1])

        gs = (C // 128, 128)
        o = pl.pallas_call(
            kern,
            in_specs=[pl.BlockSpec(memory_space=pltpu.HBM)] * 3,
            out_specs=pl.BlockSpec(memory_space=pltpu.HBM),
            out_shape=jax.ShapeDtypeStruct(xv.shape, x.dtype),
            scratch_shapes=[pltpu.VMEM((NP,) + xv.shape[1:], x.dtype),
                            pltpu.VMEM((2,) + gs, g.dtype), pltpu.VMEM((2,) + gs, jnp.float32), pltpu.SMEM((2,) + gs, jnp.float32),
                            pltpu.SemaphoreType.DMA((2,)), pltpu.SemaphoreType.DMA((2,)), pltpu.SemaphoreType.DMA((2,))],
            compiler_params=pltpu.CompilerParams(vmem_limit_bytes=(NP * 8 + 4) << 20, disable_bounds_checks=nobc),
        )(xv, g.reshape(gs), b.reshape(gs))
        return o.reshape(x.shape)
    return f


_impl = make((11, 11, 10))


@jax.jit
def pallas_standalone__groupnorm__prompt_kernel(x: jax.Array, g: jax.Array, b: jax.Array):
    return _impl(x, g, b)
```

```python
import functools

import jax
import jax.numpy as jnp
from jax import lax
import jax.experimental.pallas as pl
import jax.experimental.pallas.tpu as pltpu

_GROUPS = 32
_EPS = 1e-5
_GROUP_BLOCKS = 4
_REGION_GROUPS = 4
_REGION_BLOCKS = _GROUP_BLOCKS * _REGION_GROUPS
_HALF = _REGION_BLOCKS // 2
_TICKS = 4 * _REGION_GROUPS


def _kernel(x_hbm, g_hbm, b_hbm, o_hbm, buf, g_smem, b_smem, rsem, wsem, psem,
            *, read_lead, write_lead):
    nreg, _, cpb, H, W = x_hbm.shape
    nslot = buf.shape[0]
    C = g_hbm.shape[0]
    cpg = cpb * _GROUP_BLOCKS
    nsub = H // 8
    nline = cpb * nsub
    inv_n = 1.0 / (cpg * H * W)

    def pieces(line):
        rows = pl.ds(pl.multiple_of(lax.rem(line, nsub) * 8, 8), 8)
        c = lax.div(line, nsub)
        return [(c, rows, pl.ds(col, W // 2)) for col in (0, W // 2)]

    def start_reads(reg, slot, lo, hi):
        def body(line, carry):
            for piece in pieces(line):
                for k in range(0, _HALF, 2):
                    for queue in range(2):
                        ix = (pl.ds(queue * _HALF + k, 2),) + piece
                        pltpu.make_async_copy(
                            x_hbm.at[(reg,) + ix], buf.at[(slot,) + ix], rsem.at[slot]
                        ).start(priority=queue)
            return carry

        per = nline // _TICKS
        lax.fori_loop(lo * per, hi * per, body, 0)

    def start_writes(reg, slot, lo, hi):
        def body(i, carry):
            blocks = pl.ds(lax.div(i, nline) * _HALF, _HALF)
            for piece in pieces(lax.rem(i, nline)):
                ix = (blocks,) + piece
                pltpu.make_async_copy(
                    buf.at[(slot,) + ix], o_hbm.at[(reg,) + ix], wsem.at[slot]
                ).start()
            return carry

        per = 2 * nline // _TICKS
        lax.fori_loop(lo * per, hi * per, body, 0)

    def wait_bytes_of(view, sem):
        pltpu.make_async_copy(view, view, sem).wait()

    def wait_slots(lo, hi, sems):
        def body(slot, carry):
            wait_bytes_of(buf.at[slot], sems.at[slot])
            return carry

        lax.fori_loop(lo, hi, body, 0)

    last = nslot - 1

    def wait_last_head(sems, lead):
        wait_bytes_of(buf.at[last, :, pl.ds(1, cpb - 1)], sems.at[last])
        wait_bytes_of(buf.at[last, pl.ds(lead, _REGION_BLOCKS - lead), 0], sems.at[last])

    def wait_last_tail(sems, lead):
        wait_bytes_of(buf.at[last, pl.ds(0, lead), 0], sems.at[last])

    def normalise(reg, slot, tick):
        def tiles(blk, c):
            for r in range(0, H, 8):
                for t in range(0, W, 256):
                    ix = (slot, blk, c, slice(r, r + 8), slice(t, t + 256))
                    yield ix, buf[ix].astype(jnp.float32)

        def group(k, carry):
            blk0 = k * _GROUP_BLOCKS

            def mean_of(fn):
                def body(c, acc):
                    acc = list(acc)
                    for j in range(_GROUP_BLOCKS):
                        for n, (_, v) in enumerate(tiles(blk0 + j, c)):
                            acc[n % 2] = acc[n % 2] + fn(v)
                    return tuple(acc)

                zero = jnp.zeros((8, 256), jnp.float32)
                acc = lax.fori_loop(0, cpb, body, (zero, zero))
                return jnp.sum(acc[0] + acc[1], keepdims=True) * inv_n

            tick(4 * k)
            mu = jnp.broadcast_to(mean_of(lambda v: v), (8, 256))
            tick(4 * k + 1)
            var = mean_of(lambda v: (v - mu) * (v - mu))
            rstd = jnp.broadcast_to(lax.rsqrt(var + _EPS), (8, 256))
            chan0 = lax.rem((reg * _REGION_GROUPS + k) * cpg, C)

            def half(h, carry):
                tick(4 * k + 2 + h)

                def body(c, carry):
                    for j in range(_GROUP_BLOCKS // 2):
                        blk = h * (_GROUP_BLOCKS // 2) + j
                        chan = chan0 + blk * cpb + c
                        scale = rstd * g_smem[chan].astype(jnp.float32)
                        shift = b_smem[chan].astype(jnp.float32)
                        for ix, v in tiles(blk0 + blk, c):
                            buf[ix] = ((v - mu) * scale + shift).astype(buf.dtype)
                    return carry

                return lax.fori_loop(0, cpb, body, carry)

            return lax.fori_loop(0, 2, half, carry)

        lax.fori_loop(0, _REGION_GROUPS, group, 0)

    g_copy = pltpu.make_async_copy(g_hbm, g_smem, psem.at[0])
    b_copy = pltpu.make_async_copy(b_hbm, b_smem, psem.at[1])
    g_copy.start()
    b_copy.start()

    def phase(ph, carry):
        reg0 = ph * nslot

        def read(slot, carry):
            start_reads(reg0 + slot, slot, 0, _TICKS)
            return carry

        lax.fori_loop(0, last, read, 0)

        @pl.when(ph == 0)
        def _():
            g_copy.wait()
            b_copy.wait()

        @pl.when(ph > 0)
        def _():
            wait_last_tail(wsem, write_lead)

        wait_slots(0, 1, rsem)

        def step(slot, carry):
            def tick(i):
                @pl.when(slot == 0)
                def _():
                    start_reads(reg0 + last, last, i, i + 1)

                @pl.when(slot > 0)
                def _():
                    start_writes(reg0 + slot - 1, slot - 1, i, i + 1)

            @pl.when(slot == last)
            def _():
                wait_last_tail(rsem, read_lead)

            normalise(reg0 + slot, slot, tick)

            @pl.when(slot == 0)
            def _():
                wait_slots(1, last, rsem)
                wait_last_head(rsem, read_lead)

            return carry

        lax.fori_loop(0, nslot, step, 0)
        start_writes(reg0 + last, last, 0, _TICKS)
        wait_slots(0, last, wsem)
        wait_last_head(wsem, write_lead)
        return carry

    lax.fori_loop(0, nreg // nslot, phase, 0)
    wait_last_tail(wsem, write_lead)


def _groupnorm(x, g, b, *, nslot=8, read_lead=4, write_lead=1, interpret=False, nobc=True):
    B, C, H, W = x.shape
    nreg = B * _GROUPS // _REGION_GROUPS
    cpb = C // (_GROUPS * _GROUP_BLOCKS)
    assert C == cpb * _GROUPS * _GROUP_BLOCKS and H % 8 == 0 and W % 256 == 0
    assert cpb > 1 and cpb * (H // 8) % _TICKS == 0
    assert nslot > 1 and nreg % nslot == 0
    xv = x.reshape(nreg, _REGION_BLOCKS, cpb, H, W)
    out = pl.pallas_call(
        functools.partial(_kernel, read_lead=read_lead, write_lead=write_lead),
        in_specs=[pl.BlockSpec(memory_space=pltpu.HBM)] * 3,
        out_specs=pl.BlockSpec(memory_space=pltpu.HBM),
        out_shape=jax.ShapeDtypeStruct(xv.shape, x.dtype),
        scratch_shapes=[
            pltpu.VMEM((nslot,) + xv.shape[1:], x.dtype),
            pltpu.SMEM(g.shape, g.dtype),
            pltpu.SMEM(b.shape, b.dtype),
            pltpu.SemaphoreType.DMA((nslot,)),
            pltpu.SemaphoreType.DMA((nslot,)),
            pltpu.SemaphoreType.DMA((2,)),
        ],
        compiler_params=pltpu.CompilerParams(vmem_limit_bytes=128 << 20, disable_bounds_checks=nobc),
        interpret=interpret,
    )(xv, g, b)
    return out.reshape(x.shape)


@jax.jit
def pallas_standalone__groupnorm__prompt_kernel(
    x: jax.Array,
    g: jax.Array,
    b: jax.Array,
):
    return _groupnorm(x, g, b)
```

```python
import functools
import math

import jax
import jax.numpy as jnp
from jax import lax
import jax.experimental.pallas as pl
import jax.experimental.pallas.tpu as pltpu

_GROUPS = 32
_EPS = 1e-5
_GROUP_BLOCKS = 4
_REGION_GROUPS = 4
_REGION_BLOCKS = _GROUP_BLOCKS * _REGION_GROUPS
_HALF = _REGION_BLOCKS // 2
_TICKS = 4 * _REGION_GROUPS


def _kernel(x_hbm, g_hbm, b_hbm, o_hbm, buf, g_smem, b_smem, rsem, wsem, psem,
            *, read_lead, write_lead):
    nreg, _, nline, _, W = x_hbm.shape
    nslot = buf.shape[0]
    last = nslot - 1
    C = g_hbm.shape[0]
    cpg = C // _GROUPS
    cpb = cpg // _GROUP_BLOCKS
    lpc = nline // cpb
    inv_n = 1.0 / (_GROUP_BLOCKS * nline * 8 * W)
    aw = math.gcd(W, 512)
    pieces = [(slice(None), pl.ds(col, W // 2)) for col in (0, W // 2)]

    def start_reads(reg, slot, lo, hi):
        def body(line, carry):
            for piece in pieces:
                for k in range(0, _HALF, 2):
                    for queue in range(2):
                        ix = (pl.ds(queue * _HALF + k, 2), line) + piece
                        pltpu.make_async_copy(
                            x_hbm.at[(reg,) + ix], buf.at[(slot,) + ix], rsem.at[slot]
                        ).start(priority=queue)
            return carry

        per = nline // _TICKS
        lax.fori_loop(lo * per, hi * per, body, 0)

    def start_writes(reg, slot, lo, hi):
        def body(i, carry):
            upper = (i >= nline).astype(jnp.int32)
            for piece in pieces:
                ix = (pl.ds(upper * _HALF, _HALF), i - upper * nline) + piece
                pltpu.make_async_copy(
                    buf.at[(slot,) + ix], o_hbm.at[(reg,) + ix], wsem.at[slot]
                ).start()
            return carry

        per = 2 * nline // _TICKS
        lax.fori_loop(lo * per, hi * per, body, 0)

    def wait_bytes_of(view, sem):
        pltpu.make_async_copy(view, view, sem).wait()

    def wait_slot(slot, sems):
        wait_bytes_of(buf.at[slot], sems.at[slot])

    def wait_last_head(sems, lead):
        wait_bytes_of(buf.at[last, :, pl.ds(lpc, nline - lpc)], sems.at[last])
        rest = pl.ds(lead, _REGION_BLOCKS - lead)
        wait_bytes_of(buf.at[last, rest, pl.ds(0, lpc)], sems.at[last])

    def wait_last_tail(sems, lead):
        wait_bytes_of(buf.at[last, pl.ds(0, lead), pl.ds(0, lpc)], sems.at[last])

    def normalise(reg, slot, tick):
        def group(k, carry):
            blk0 = k * _GROUP_BLOCKS

            def mean_of(fn):
                def body(c, acc):
                    for j in range(_GROUP_BLOCKS):
                        for r in range(lpc):
                            v = buf[slot, blk0 + j, c * lpc + r]
                            for t in range(0, W, aw):
                                acc = acc + fn(v[:, t:t + aw].astype(jnp.float32))
                    return acc

                acc = lax.fori_loop(0, cpb, body, jnp.zeros((8, aw), jnp.float32))
                return jnp.sum(acc, keepdims=True) * inv_n

            tick(4 * k)
            mu = mean_of(lambda v: v)
            tick(4 * k + 1)
            var = mean_of(lambda v: (v - mu) * (v - mu))
            rstd = lax.rsqrt(var + _EPS)
            chan0 = lax.rem((reg * _REGION_GROUPS + k) * cpg, C)

            def half(h, carry):
                tick(4 * k + 2 + h)

                def body(c, carry):
                    for j in range(_GROUP_BLOCKS // 2):
                        blk = h * (_GROUP_BLOCKS // 2) + j
                        chan = chan0 + blk * cpb + c
                        scale = rstd * g_smem[chan].astype(jnp.float32)
                        shift = b_smem[chan].astype(jnp.float32)
                        for r in range(lpc):
                            ix = (slot, blk0 + blk, c * lpc + r)
                            v = buf[ix].astype(jnp.float32)
                            buf[ix] = ((v - mu) * scale + shift).astype(buf.dtype)
                    return carry

                return lax.fori_loop(0, cpb, body, carry)

            return lax.fori_loop(0, 2, half, carry)

        lax.fori_loop(0, _REGION_GROUPS, group, 0)

    g_copy = pltpu.make_async_copy(g_hbm, g_smem, psem.at[0])
    b_copy = pltpu.make_async_copy(b_hbm, b_smem, psem.at[1])
    g_copy.start()
    b_copy.start()

    def phase(ph, carry):
        reg0 = ph * nslot

        def read(slot, carry):
            start_reads(reg0 + slot, slot, 0, _TICKS)

            @pl.when(slot > 0)
            def _():
                wait_slot(slot - 1, rsem)

            return carry

        lax.fori_loop(0, last, read, 0)

        @pl.when(ph == 0)
        def _():
            g_copy.wait()
            b_copy.wait()

        @pl.when(ph > 0)
        def _():
            wait_last_tail(wsem, write_lead)

        def step(slot, carry):
            def tick(i):
                @pl.when(slot == 0)
                def _():
                    start_reads(reg0 + last, last, i, i + 1)

                @pl.when(slot > 0)
                def _():
                    start_writes(reg0 + slot - 1, slot - 1, i, i + 1)

            @pl.when(slot == last)
            def _():
                wait_last_tail(rsem, read_lead)

            normalise(reg0 + slot, slot, tick)

            @pl.when(slot == 0)
            def _():
                wait_slot(last - 1, rsem)
                wait_last_head(rsem, read_lead)

            @pl.when(slot > 1)
            def _():
                wait_slot(slot - 2, wsem)

            return carry

        lax.fori_loop(0, nslot, step, 0)
        start_writes(reg0 + last, last, 0, _TICKS)
        wait_slot(last - 1, wsem)
        wait_last_head(wsem, write_lead)
        return carry

    lax.fori_loop(0, nreg // nslot, phase, 0)
    wait_last_tail(wsem, write_lead)


def _groupnorm(x, g, b, *, nslot=8, read_lead=3, write_lead=1, interpret=False):
    B, C, H, W = x.shape
    nreg = B * _GROUPS // _REGION_GROUPS
    cpb = C // (_GROUPS * _GROUP_BLOCKS)
    nline = cpb * H // 8
    assert C == cpb * _GROUPS * _GROUP_BLOCKS and H % 8 == 0 and W % 256 == 0
    assert cpb > 1 and nline % _TICKS == 0
    assert nslot > 2 and nreg % nslot == 0
    xv = x.reshape(nreg, _REGION_BLOCKS, nline, 8, W)
    out = pl.pallas_call(
        functools.partial(_kernel, read_lead=read_lead, write_lead=write_lead),
        in_specs=[pl.BlockSpec(memory_space=pltpu.HBM)] * 3,
        out_specs=pl.BlockSpec(memory_space=pltpu.HBM),
        out_shape=jax.ShapeDtypeStruct(xv.shape, x.dtype),
        scratch_shapes=[
            pltpu.VMEM((nslot,) + xv.shape[1:], x.dtype),
            pltpu.SMEM(g.shape, g.dtype),
            pltpu.SMEM(b.shape, b.dtype),
            pltpu.SemaphoreType.DMA((nslot,)),
            pltpu.SemaphoreType.DMA((nslot,)),
            pltpu.SemaphoreType.DMA((2,)),
        ],
        compiler_params=pltpu.CompilerParams(
            vmem_limit_bytes=128 << 20, disable_bounds_checks=True),
        interpret=interpret,
    )(xv, g, b)
    return out.reshape(x.shape)


@jax.jit
def pallas_standalone__groupnorm__prompt_kernel(
    x: jax.Array,
    g: jax.Array,
    b: jax.Array,
):
    return _groupnorm(x, g, b)
```

```python
import functools
import math

import jax
import jax.numpy as jnp
from jax import lax
import jax.experimental.pallas as pl
import jax.experimental.pallas.tpu as pltpu

_GROUPS = 32
_EPS = 1e-5
_GROUP_BLOCKS = 4
_REGION_GROUPS = 4
_REGION_BLOCKS = _GROUP_BLOCKS * _REGION_GROUPS
_HALF = _REGION_BLOCKS // 2
_TICKS = 4 * _REGION_GROUPS


def _kernel(x_hbm, g_hbm, b_hbm, o_hbm, buf, g_smem, b_smem, rsem, wsem, psem,
            *, read_lead, write_lead):
    nreg, _, nline, _, W = x_hbm.shape
    nslot = buf.shape[0]
    last = nslot - 1
    C = g_hbm.shape[0]
    cpg = C // _GROUPS
    cpb = cpg // _GROUP_BLOCKS
    lpc = nline // cpb
    inv_n = 1.0 / (_GROUP_BLOCKS * nline * 8 * W)
    aw = math.gcd(W, 512)
    pieces = [(slice(None), pl.ds(col, W // 2)) for col in (0, W // 2)]

    def start_reads(reg, slot, lo, hi):
        def body(line, carry):
            for piece in pieces:
                for k in range(0, _HALF, 2):
                    for queue in range(2):
                        ix = (pl.ds(queue * _HALF + k, 2), line) + piece
                        pltpu.make_async_copy(
                            x_hbm.at[(reg,) + ix], buf.at[(slot,) + ix], rsem.at[slot]
                        ).start(priority=queue)
            return carry

        per = nline // _TICKS
        lax.fori_loop(lo * per, hi * per, body, 0)

    def start_writes(reg, slot, lo, hi):
        def body(i, carry):
            upper = (i >= nline).astype(jnp.int32)
            for piece in pieces:
                ix = (pl.ds(upper * _HALF, _HALF), i - upper * nline) + piece
                pltpu.make_async_copy(
                    buf.at[(slot,) + ix], o_hbm.at[(reg,) + ix], wsem.at[slot]
                ).start()
            return carry

        per = 2 * nline // _TICKS
        lax.fori_loop(lo * per, hi * per, body, 0)

    def wait_bytes_of(view, sem):
        pltpu.make_async_copy(view, view, sem).wait()

    def wait_slot(slot, sems):
        wait_bytes_of(buf.at[slot], sems.at[slot])

    def wait_last_head(sems, lead):
        wait_bytes_of(buf.at[last, :, pl.ds(lpc, nline - lpc)], sems.at[last])
        rest = pl.ds(lead, _REGION_BLOCKS - lead)
        wait_bytes_of(buf.at[last, rest, pl.ds(0, lpc)], sems.at[last])

    def wait_last_tail(sems, lead):
        wait_bytes_of(buf.at[last, pl.ds(0, lead), pl.ds(0, lpc)], sems.at[last])

    def normalise(reg, slot, tick):
        def group(k, carry):
            blk0 = k * _GROUP_BLOCKS

            def mean_of(fn):
                def body(c, acc):
                    for j in range(_GROUP_BLOCKS):
                        v = buf[slot, blk0 + j, pl.ds(c * lpc, lpc)]
                        for r in range(lpc):
                            for t in range(0, W, aw):
                                acc = acc + fn(v[r, :, t:t + aw].astype(jnp.float32))
                    return acc

                acc = lax.fori_loop(0, cpb, body, jnp.zeros((8, aw), jnp.float32))
                return jnp.sum(acc, keepdims=True) * inv_n

            tick(4 * k)
            mu = mean_of(lambda v: v)
            tick(4 * k + 1)
            var = mean_of(lambda v: (v - mu) * (v - mu))
            rstd = lax.rsqrt(var + _EPS)
            chan0 = lax.rem((reg * _REGION_GROUPS + k) * cpg, C)

            def half(h, carry):
                tick(4 * k + 2 + h)

                def body(c, carry):
                    for j in range(_GROUP_BLOCKS // 2):
                        blk = h * (_GROUP_BLOCKS // 2) + j
                        chan = chan0 + blk * cpb + c
                        scale = rstd * g_smem[chan].astype(jnp.float32)
                        shift = b_smem[chan].astype(jnp.float32)
                        ix = (slot, blk0 + blk, pl.ds(c * lpc, lpc))
                        v = buf[ix]
                        buf[ix] = jnp.stack([
                            ((v[r].astype(jnp.float32) - mu) * scale + shift).astype(v.dtype)
                            for r in range(lpc)
                        ])
                    return carry

                return lax.fori_loop(0, cpb, body, carry)

            return lax.fori_loop(0, 2, half, carry)

        lax.fori_loop(0, _REGION_GROUPS, group, 0)

    g_copy = pltpu.make_async_copy(g_hbm, g_smem, psem.at[0])
    b_copy = pltpu.make_async_copy(b_hbm, b_smem, psem.at[1])
    g_copy.start()
    b_copy.start()

    def phase(ph, carry):
        reg0 = ph * nslot

        def read(slot, carry):
            start_reads(reg0 + slot, slot, 0, _TICKS)

            @pl.when(slot > 0)
            def _():
                wait_slot(slot - 1, rsem)

            return carry

        lax.fori_loop(0, last, read, 0)

        @pl.when(ph == 0)
        def _():
            g_copy.wait()
            b_copy.wait()

        @pl.when(ph > 0)
        def _():
            wait_last_tail(wsem, write_lead)

        def step(slot, carry):
            def tick(i):
                @pl.when(slot == 0)
                def _():
                    start_reads(reg0 + last, last, i, i + 1)

                @pl.when(slot > 0)
                def _():
                    start_writes(reg0 + slot - 1, slot - 1, i, i + 1)

            @pl.when(slot == last)
            def _():
                wait_last_tail(rsem, read_lead)

            normalise(reg0 + slot, slot, tick)

            @pl.when(slot == 0)
            def _():
                wait_slot(last - 1, rsem)
                wait_last_head(rsem, read_lead)

            @pl.when(slot > 1)
            def _():
                wait_slot(slot - 2, wsem)

            return carry

        lax.fori_loop(0, nslot, step, 0)
        start_writes(reg0 + last, last, 0, _TICKS)
        wait_slot(last - 1, wsem)
        wait_last_head(wsem, write_lead)
        return carry

    lax.fori_loop(0, nreg // nslot, phase, 0)
    wait_last_tail(wsem, write_lead)


def _groupnorm(x, g, b, *, nslot=8, read_lead=3, write_lead=1, interpret=False):
    B, C, H, W = x.shape
    nreg = B * _GROUPS // _REGION_GROUPS
    cpb = C // (_GROUPS * _GROUP_BLOCKS)
    nline = cpb * H // 8
    assert C == cpb * _GROUPS * _GROUP_BLOCKS and H % 8 == 0 and W % 256 == 0
    assert cpb > 1 and nline % _TICKS == 0
    assert nslot > 2 and nreg % nslot == 0
    xv = x.reshape(nreg, _REGION_BLOCKS, nline, 8, W)
    out = pl.pallas_call(
        functools.partial(_kernel, read_lead=read_lead, write_lead=write_lead),
        in_specs=[pl.BlockSpec(memory_space=pltpu.HBM)] * 3,
        out_specs=pl.BlockSpec(memory_space=pltpu.HBM),
        out_shape=jax.ShapeDtypeStruct(xv.shape, x.dtype),
        scratch_shapes=[
            pltpu.VMEM((nslot,) + xv.shape[1:], x.dtype),
            pltpu.SMEM(g.shape, g.dtype),
            pltpu.SMEM(b.shape, b.dtype),
            pltpu.SemaphoreType.DMA((nslot,)),
            pltpu.SemaphoreType.DMA((nslot,)),
            pltpu.SemaphoreType.DMA((2,)),
        ],
        compiler_params=pltpu.CompilerParams(
            vmem_limit_bytes=128 << 20, disable_bounds_checks=True),
        interpret=interpret,
    )(xv, g, b)
    return out.reshape(x.shape)


@jax.jit
def pallas_standalone__groupnorm__prompt_kernel(
    x: jax.Array,
    g: jax.Array,
    b: jax.Array,
):
    return _groupnorm(x, g, b)
```

```python
import math

import jax
import jax.numpy as jnp
from jax import lax
import jax.experimental.pallas as pl
import jax.experimental.pallas.tpu as pltpu

_GROUPS = 32
_EPS = 1e-5
_GROUP_BLOCKS = 4
_REGION_GROUPS = 4
_REGION_BLOCKS = _GROUP_BLOCKS * _REGION_GROUPS
_HALF = _REGION_BLOCKS // 2
_TICKS = 4 * _REGION_GROUPS
_LEAD = 2


def _kernel(x_hbm, g_hbm, b_hbm, o_hbm, buf, g_smem, b_smem, rsem, wsem, psem):
    nreg, _, nline, _, W = x_hbm.shape
    nslot = buf.shape[0]
    last = nslot - 1
    head = nline - _LEAD
    C = g_hbm.shape[0]
    cpg = C // _GROUPS
    cpb = cpg // _GROUP_BLOCKS
    lpc = nline // cpb
    inv_n = 1.0 / (_GROUP_BLOCKS * nline * 8 * W)
    aw = math.gcd(W, 512)
    pieces = [(slice(None), pl.ds(col, W // 2)) for col in (0, W // 2)]

    def start_reads(reg, slot, lo, hi, sem_of_line):
        def body(line, carry):
            sem = rsem.at[sem_of_line(line)]
            for piece in pieces:
                for k in range(0, _HALF, 2):
                    for queue in range(2):
                        ix = (pl.ds(queue * _HALF + k, 2), line) + piece
                        pltpu.make_async_copy(
                            x_hbm.at[(reg,) + ix], buf.at[(slot,) + ix], sem
                        ).start(priority=queue)
            return carry

        per = nline // _TICKS
        lax.fori_loop(lo * per, hi * per, body, 0)

    def start_writes(reg, slot, lo, hi):
        def body(i, carry):
            upper = (i >= nline).astype(jnp.int32)
            for piece in pieces:
                ix = (pl.ds(upper * _HALF, _HALF), i - upper * nline) + piece
                pltpu.make_async_copy(
                    buf.at[(slot,) + ix], o_hbm.at[(reg,) + ix], wsem.at[slot]
                ).start()
            return carry

        per = 2 * nline // _TICKS
        lax.fori_loop(lo * per, hi * per, body, 0)

    def wait_filled(view, sem):
        pltpu.make_async_copy(view, view, sem).wait()

    def wait_slot(slot, sems):
        wait_filled(buf.at[slot], sems.at[slot])

    def normalise(reg, slot, tick):
        def group(k, carry):
            blk0 = k * _GROUP_BLOCKS

            def mean_of(fn):
                def body(c, acc):
                    for j in range(_GROUP_BLOCKS):
                        v = buf[slot, blk0 + j, pl.ds(c * lpc, lpc)]
                        for r in range(lpc):
                            for t in range(0, W, aw):
                                acc = acc + fn(v[r, :, t:t + aw].astype(jnp.float32))
                    return acc

                acc = lax.fori_loop(0, cpb, body, jnp.zeros((8, aw), jnp.float32))
                return jnp.sum(acc, keepdims=True) * inv_n

            tick(4 * k)
            mu = mean_of(lambda v: v)
            tick(4 * k + 1)
            var = mean_of(lambda v: (v - mu) * (v - mu))
            rstd = lax.rsqrt(var + _EPS)
            chan0 = lax.rem((reg * _REGION_GROUPS + k) * cpg, C)

            def half(h, carry):
                tick(4 * k + 2 + h)

                def body(c, carry):
                    for j in range(_GROUP_BLOCKS // 2):
                        blk = h * (_GROUP_BLOCKS // 2) + j
                        chan = chan0 + blk * cpb + c
                        scale = rstd * g_smem[chan].astype(jnp.float32)
                        shift = b_smem[chan].astype(jnp.float32)
                        ix = (slot, blk0 + blk, pl.ds(c * lpc, lpc))
                        v = buf[ix]
                        buf[ix] = jnp.stack([
                            ((v[r].astype(jnp.float32) - mu) * scale + shift).astype(v.dtype)
                            for r in range(lpc)
                        ])
                    return carry

                return lax.fori_loop(0, cpb, body, carry)

            return lax.fori_loop(0, 2, half, carry)

        lax.fori_loop(0, _REGION_GROUPS, group, 0)

    g_copy = pltpu.make_async_copy(g_hbm, g_smem, psem.at[0])
    b_copy = pltpu.make_async_copy(b_hbm, b_smem, psem.at[1])
    g_copy.start()
    b_copy.start()

    def phase(ph, carry):
        reg0 = ph * nslot

        def read(slot, carry):
            start_reads(reg0 + slot, slot, 0, _TICKS, lambda line: slot)

            @pl.when(slot > 0)
            def _():
                wait_slot(slot - 1, rsem)

            return carry

        lax.fori_loop(0, last, read, 0)

        @pl.when(ph == 0)
        def _():
            g_copy.wait()
            b_copy.wait()

        def step(slot, carry):
            def tick(i):
                @pl.when(slot == 0)
                def _():
                    start_reads(reg0 + last, last, i, i + 1,
                                lambda line: last + (line >= head).astype(jnp.int32))

                @pl.when(slot > 0)
                def _():
                    start_writes(reg0 + slot - 1, slot - 1, i, i + 1)

            @pl.when(slot == last)
            def _():
                wait_filled(buf.at[last, :, pl.ds(head, _LEAD)], rsem.at[nslot])

            normalise(reg0 + slot, slot, tick)

            @pl.when(slot == 0)
            def _():
                wait_slot(last - 1, rsem)
                wait_filled(buf.at[last, :, pl.ds(0, head)], rsem.at[last])

            @pl.when(slot > 1)
            def _():
                wait_slot(slot - 2, wsem)

            return carry

        lax.fori_loop(0, nslot, step, 0)
        start_writes(reg0 + last, last, 0, _TICKS)
        wait_slot(last - 1, wsem)
        wait_slot(last, wsem)
        return carry

    lax.fori_loop(0, nreg // nslot, phase, 0)


def _groupnorm(x, g, b, *, nslot=8, interpret=False):
    B, C, H, W = x.shape
    nreg = B * _GROUPS // _REGION_GROUPS
    cpb = C // (_GROUPS * _GROUP_BLOCKS)
    nline = cpb * H // 8
    assert C == cpb * _GROUPS * _GROUP_BLOCKS and H % 8 == 0 and W % 256 == 0
    assert nline % _TICKS == 0
    assert nslot > 2 and nreg % nslot == 0
    xv = x.reshape(nreg, _REGION_BLOCKS, nline, 8, W)
    out = pl.pallas_call(
        _kernel,
        in_specs=[pl.BlockSpec(memory_space=pltpu.HBM)] * 3,
        out_specs=pl.BlockSpec(memory_space=pltpu.HBM),
        out_shape=jax.ShapeDtypeStruct(xv.shape, x.dtype),
        scratch_shapes=[
            pltpu.VMEM((nslot,) + xv.shape[1:], x.dtype),
            pltpu.SMEM(g.shape, g.dtype),
            pltpu.SMEM(b.shape, b.dtype),
            pltpu.SemaphoreType.DMA((nslot + 1,)),
            pltpu.SemaphoreType.DMA((nslot,)),
            pltpu.SemaphoreType.DMA((2,)),
        ],
        compiler_params=pltpu.CompilerParams(
            vmem_limit_bytes=128 << 20, disable_bounds_checks=True),
        interpret=interpret,
    )(xv, g, b)
    return out.reshape(x.shape)


@jax.jit
def pallas_standalone__groupnorm__prompt_kernel(
    x: jax.Array,
    g: jax.Array,
    b: jax.Array,
):
    return _groupnorm(x, g, b)
```
